```python
import jax
import jax.numpy as jnp

def _softmax(x, axis=-1):
    return jax.nn.softmax(x, axis=axis)
def _gelu(x):
    return jax.nn.gelu(x, approximate=True)
def _silu(x):
    return jax.nn.silu(x)
def _sigmoid(x):
    return jax.nn.sigmoid(x)
def _layernorm(x, axis=-1, eps=1e-5):
    m = jnp.mean(x, axis=axis, keepdims=True)
    v = jnp.var(x, axis=axis, keepdims=True)
    return (x - m) / jnp.sqrt(v + eps)
def _scatter_add(tgt, idx, src, axis=0):
    return tgt.at[idx].add(src)
def _segment_sum(src, seg, n):
    return jax.ops.segment_sum(src, seg, n)
class _Rng:
    def __init__(self, key):
        self._k = key
    def _next(self):
        self._k, sub = jax.random.split(self._k)
        return sub
    def normal(self, shape):
        return jax.random.normal(self._next(), shape, dtype=jnp.bfloat16)
    def randint(self, lo, hi, shape):
        return jax.random.randint(self._next(), shape, lo, hi, dtype=jnp.int32)
    def uniform(self, shape, lo=0.0, hi=1.0):
        return jax.random.uniform(self._next(), shape, jnp.bfloat16, lo, hi)
    def permutation(self, n):
        return jax.random.permutation(self._next(), n)


kernel_name = 'sequential_preLN__sliding_block_cached__moe_arch_mod__decode'

def setup_inputs():
    _rng = _Rng(jax.random.key(int.from_bytes(__import__("os").urandom(4), "little")))
    _w = (lambda a: (lambda t: t.astype(jnp.bfloat16) if jnp.issubdtype(t.dtype, jnp.floating) else t)(jnp.asarray(a)))
    def _A_setup():
        B, Sq, D = 1, 1, 640
        Hq, Hkv, Sk, Dh = 32, 32, 32768, 192
        assert Hq % Hkv == 0, (Hq, Hkv)
        return {
            "x": _w((lambda *s: _rng.normal(s) * 0.05)(B, Sq, D)),
            "k_cache": _w((lambda *s: _rng.normal(s) * 0.05)(B, Hkv, Sk, Dh)),
            "v_cache": _w((lambda *s: _rng.normal(s) * 0.05)(B, Hkv, Sk, Dh)),
            "wq": _w((lambda *s: _rng.normal(s) * 0.05)(D, Hq * Dh) * (D ** -0.5)),
            "wo": _w((lambda *s: _rng.normal(s) * 0.05)(Hq * Dh, D) * ((Hq * Dh) ** -0.5)),
        }
    _A_in = _A_setup()

    def _B_setup():
        B, S, D, F, C = 1, 1, 640, 1536, 1
        return {
            "x": _w((lambda *s: _rng.normal(s) * 0.05)(B, S, D)),
            "w_r": _w((lambda *s: _rng.normal(s) * 0.05)(D)),
            "w_gate": _w((lambda *s: _rng.normal(s) * 0.05)(D, F)),
            "w_up": _w((lambda *s: _rng.normal(s) * 0.05)(D, F)),
            "w_down": _w((lambda *s: _rng.normal(s) * 0.05)(F, D)),
        }
    _B_in = _B_setup()

    return {
        "A_x": _A_in["x"],
        "A_k_cache": _A_in["k_cache"],
        "A_v_cache": _A_in["v_cache"],
        "A_wq": _A_in["wq"],
        "A_wo": _A_in["wo"],
        "B_x": _B_in["x"],
        "B_w_r": _B_in["w_r"],
        "B_w_gate": _B_in["w_gate"],
        "B_w_up": _B_in["w_up"],
        "B_w_down": _B_in["w_down"],
    }

def reference(A_x, A_k_cache, A_v_cache, A_wq, A_wo, B_x, B_w_r, B_w_gate, B_w_up, B_w_down):
    def _A_ref(x, k_cache, v_cache, wq, wo):
        B, Sq, D = x.shape
        Hq, Dh = 32, 192
        Hkv, Sk = k_cache.shape[1], k_cache.shape[2]
        W = min(4096, max(256, Sk // 4))
        rep = Hq // Hkv
        q = (lambda x, *d: x.transpose(*d))((x @ wq).reshape(B, Sq, Hq, Dh), 0, 2, 1, 3)
        k = jnp.repeat(k_cache[:, :, Sk - W:, :], rep, axis=1)
        v = jnp.repeat(v_cache[:, :, Sk - W:, :], rep, axis=1)
        scores = jnp.einsum("bhqd,bhkd->bhqk", q, k) * (Dh ** -0.5)
        p = _softmax(scores, axis=-1)
        o = jnp.einsum("bhqk,bhkd->bhqd", p, v)
        return (lambda x, *d: x.transpose(*d))(o, 0, 2, 1, 3).reshape(B, Sq, Hq * Dh) @ wo

    def _B_ref(x, w_r, w_gate, w_up, w_down):
        B, S, D = x.shape
        C = 1
        r = x @ w_r
        idx = jnp.argsort(-r, axis=-1)[:, :C]
        idx_e = jnp.repeat(idx.reshape(B, C, 1), D, axis=2)
        x_sel = jnp.take_along_axis(x, idx_e, axis=1)
        g = _silu(x_sel @ w_gate)
        u = x_sel @ w_up
        y = (g * u) @ w_down
        r_sel = _sigmoid(jnp.take_along_axis(r, idx, axis=1))
        y = y * r_sel.reshape(B, C, 1)
        b_off = (jnp.arange(B) * S).reshape(B, 1)
        flat_idx = (idx + b_off).reshape(B * C)
        zero = (x * 0.0).reshape(B * S, D)
        upd = _scatter_add(zero, flat_idx, y.reshape(B * C, D), axis=0)
        return x + upd.reshape(B, S, D)

    x = A_x
    h = x + _A_ref(_layernorm(x, axis=-1), A_k_cache, A_v_cache, A_wq, A_wo)
    h2 = h + _B_ref(_layernorm(h, axis=-1), B_w_r, B_w_gate, B_w_up, B_w_down)
    return h2
```

```python
from functools import partial

import jax
import jax.numpy as jnp
from jax import lax
import jax.experimental.pallas as pl
import jax.experimental.pallas.tpu as pltpu

EPS = 1e-5
GROUPS, PIECES = 4, 6
HALF = GROUPS * PIECES
KV_ROWS, KV_COLS = 32, 512
NBUF = 3
DOWN_ROWS = 32
DOWN_EDGES = (0, 512, 1024, 1408, 1536)


def _layernorm(x):
    m = jnp.mean(x, axis=-1, keepdims=True)
    d = x - m
    v = jnp.mean(d * d, axis=-1, keepdims=True)
    return d / jnp.sqrt(v + EPS)


def _kernel(x_hbm, kt_hbm, vt_hbm, wq_hbm, wo_hbm, wr_hbm, wg_hbm, wu_hbm, wd_hbm,
            o_ref,
            x_s, wr_s, wq_s, wo_s, wg_s, wu_s, wd_s, k_s, v_s, q_s, oh_s, p_s, l_s,
            sem_k, sem_v, sem_w, sem_d):
    _, H, Dh, Sk = kt_hbm.shape
    W = k_s.shape[-1]
    D = x_hbm.shape[-1]
    F = wd_hbm.shape[0]
    f32, bf16 = jnp.float32, jnp.bfloat16

    def kv_copy(src, dst, sem, h, b, g, i):
        c = pl.multiple_of((b * GROUPS + g) * KV_COLS, KV_COLS)
        rows = pl.ds(i * KV_ROWS, KV_ROWS)
        return pltpu.make_async_copy(src.at[0, h, rows, pl.ds(Sk - W + c, KV_COLS)],
                                     dst.at[h % NBUF, rows, pl.ds(c, KV_COLS)], sem.at[h % NBUF])

    k_copy = partial(kv_copy, kt_hbm, k_s, sem_k)
    v_copy = partial(kv_copy, vt_hbm, v_s, sem_v)

    def wq_copy(half, b, g, i):
        r = pl.multiple_of((b * 2 + g // 2) * 8, 8)
        c = pl.multiple_of(((g % 2) * PIECES + i) * 512, 512)
        idx = (pl.ds(half * 5, 5), pl.ds(r, 8), pl.ds(c, 512))
        return pltpu.make_async_copy(wq_hbm.at[idx], wq_s.at[idx], sem_w.at[0])

    def wo_copy(half, b, g, i):
        r = pl.multiple_of((((b % 2) * GROUPS + g) * PIECES + i) * 8, 8)
        idx = (b // 2, pl.ds(half * 4, 4), pl.ds(r, 8), slice(None))
        return pltpu.make_async_copy(wo_hbm.at[idx], wo_s.at[idx], sem_w.at[1 + b // 2])

    def gu_copy(src, dst, b, g, i):
        r = pl.multiple_of(((b * GROUPS + g) * 2 + i // 3) * 8, 8)
        idx = (slice(None), pl.ds(r, 8), pl.ds(pl.multiple_of((i % 3) * 512, 512), 512))
        return pltpu.make_async_copy(src.at[idx], dst.at[idx], sem_w.at[3])

    wg_copy = partial(gu_copy, wg_hbm, wg_s)
    wu_copy = partial(gu_copy, wu_hbm, wu_s)

    def wd_copy(p):
        r = pl.multiple_of(p * DOWN_ROWS, DOWN_ROWS)
        chunk = sum((r >= e).astype(jnp.int32) for e in DOWN_EDGES[1:-1])
        idx = (pl.ds(r, DOWN_ROWS), slice(None))
        return pltpu.make_async_copy(wd_hbm.at[idx], wd_s.at[idx], sem_d.at[chunk])

    def landed(dst, sem):
        pltpu.make_async_copy(dst, dst, sem).wait()

    def half_round(low, high):
        def group(g, _):
            for i in range(PIECES):
                low(g, i).start(priority=1)
                if high is not None:
                    high(g, i).start(priority=0)
        lax.fori_loop(0, GROUPS, group, None)

    def q_proj(g0, g1):
        def body(g, _):
            c = pl.multiple_of(g * 4 * Dh, 128)
            q = jnp.dot(xn, wq_s[:, :, pl.ds(c, 4 * Dh)].reshape(D, 4 * Dh),
                        preferred_element_type=f32)
            for j in range(4):
                q_s[g * 4 + j] = q[:, j * Dh:(j + 1) * Dh].astype(bf16)
        lax.fori_loop(g0, g1, body, None)

    def scores(h):
        slot = h % NBUF
        landed(k_s.at[slot], sem_k.at[slot])
        s = jnp.dot(q_s[h], k_s[slot], preferred_element_type=f32) * Dh ** -0.5
        e = jnp.exp(s - jnp.max(s, axis=-1, keepdims=True))
        l_s[...] = jnp.broadcast_to(jnp.sum(e, axis=-1, keepdims=True), l_s.shape)
        p_s[...] = e.astype(bf16)

    def values(h):
        slot = h % NBUF
        landed(v_s.at[slot], sem_v.at[slot])
        a = lax.dot_general(p_s[...], v_s[slot], (((1,), (1,)), ((), ())),
                            preferred_element_type=f32)
        oh_s[h] = (a / l_s[:, :1]).astype(bf16)

    def o_proj(t, g0, g1, y):
        def body(g, y):
            for j in range(2):
                y = y + jnp.dot(oh_s[t * 16 + g * 2 + j], wo_s[t, g, j * Dh:(j + 1) * Dh, :],
                                preferred_element_type=f32)
            return y
        return lax.fori_loop(g0, g1, body, y)

    x_copy = pltpu.make_async_copy(x_hbm, x_s, sem_w.at[4])
    wr_copy = pltpu.make_async_copy(wr_hbm, wr_s, sem_w.at[5])

    half_round(partial(wq_copy, 0, 0), None)
    x_copy.start()
    wr_copy.start()
    lax.fori_loop(0, 3, lambda b, _: half_round(partial(wq_copy, 0, b + 1),
                                                partial(wq_copy, 1, b)), None)
    half_round(partial(k_copy, 0, 0), partial(wq_copy, 1, 3))
    half_round(partial(k_copy, 0, 1), partial(v_copy, 0, 0))
    x_copy.wait()
    wr_copy.wait()
    x = x_s[0].astype(f32)
    xn = jnp.broadcast_to(_layernorm(x), (8, D)).astype(bf16)
    half_round(partial(k_copy, 1, 0), partial(v_copy, 0, 1))
    landed(wq_s, sem_w.at[0])
    q_proj(0, 4)
    half_round(partial(k_copy, 1, 1), partial(v_copy, 1, 0))
    q_proj(4, 8)

    def head_round(j, _):
        half_round(partial(k_copy, j + 1, 0), partial(v_copy, j, 1))
        scores(j - 1)
        half_round(partial(k_copy, j + 1, 1), partial(v_copy, j + 1, 0))
        values(j - 1)
    lax.fori_loop(1, H - 1, head_round, None)

    half_round(partial(wo_copy, 0, 0), partial(v_copy, H - 1, 1))

    def last_heads(t, _):
        scores(H - 2 + t)
        half_round(partial(wo_copy, 0, 2 * t + 1), partial(wo_copy, 1, 2 * t))
        values(H - 2 + t)

        @pl.when(t == 0)
        def _():
            half_round(partial(wo_copy, 0, 2), partial(wo_copy, 1, 1))
    lax.fori_loop(0, 2, last_heads, None)

    landed(wo_s.at[0], sem_w.at[1])
    y = o_proj(0, 0, 4, jnp.zeros((8, D), f32))
    half_round(partial(wg_copy, 0), partial(wo_copy, 1, 3))
    y = o_proj(0, 4, 8, y)
    half_round(partial(wg_copy, 1), partial(wu_copy, 0))

    shared = (F // DOWN_ROWS - HALF) // 2

    def last_up(n, _):
        wd_copy(jnp.where(n < shared, 2 * n, n + shared)).start(priority=1)
        wu_copy(1, n // PIECES, n % PIECES).start(priority=0)
    lax.fori_loop(0, HALF, last_up, None)
    landed(wo_s.at[1], sem_w.at[2])
    y = o_proj(1, 0, 4, y)

    def last_down(n, _):
        wd_copy(n + HALF + shared).start(priority=1)
        wd_copy(2 * n + 1).start(priority=0)
    lax.fori_loop(0, shared, last_down, None)
    y = o_proj(1, 4, 8, y)

    hres = x + y[0:1, :]
    hn = _layernorm(hres)
    wr = wr_s[...].astype(f32).reshape(1, D)
    gate = jax.nn.sigmoid(jnp.sum(hn * wr, axis=-1, keepdims=True))
    hb = jnp.broadcast_to(hn, (8, D)).astype(bf16)

    landed(wg_s, sem_w.at[3])
    landed(wu_s, sem_w.at[3])
    g = jnp.dot(hb, wg_s[...].reshape(D, F), preferred_element_type=f32)
    u = jnp.dot(hb, wu_s[...].reshape(D, F), preferred_element_type=f32)
    gu = (g * jax.nn.sigmoid(g) * u).astype(bf16)
    y = jnp.zeros((8, D), f32)
    for c, (r0, r1) in enumerate(zip(DOWN_EDGES[:-1], DOWN_EDGES[1:])):
        landed(wd_s.at[pl.ds(r0, r1 - r0)], sem_d.at[c])
        y = y + jnp.dot(gu[:, r0:r1], wd_s[r0:r1, :], preferred_element_type=f32)
    o_ref[0] = (hres + (hn + y[:1] * gate)).astype(o_ref.dtype)


@jax.jit
def pallas_sequential_preLN__sliding_block_cached__moe_arch_mod__decode_kernel(
    A_x: jax.Array,
    A_k_cache: jax.Array,
    A_v_cache: jax.Array,
    A_wq: jax.Array,
    A_wo: jax.Array,
    B_x: jax.Array,
    B_w_r: jax.Array,
    B_w_gate: jax.Array,
    B_w_up: jax.Array,
    B_w_down: jax.Array,
):
    del B_x
    _, H, Sk, Dh = A_k_cache.shape
    D = A_x.shape[-1]
    F = B_w_gate.shape[-1]
    W = min(4096, max(256, Sk // 4))
    kt = jnp.transpose(A_k_cache, (0, 1, 3, 2))
    vt = jnp.transpose(A_v_cache, (0, 1, 3, 2))
    wq = A_wq.reshape(10, D // 10, H * Dh)
    wo = A_wo.reshape(2, 8, H * Dh // 16, D)
    wg = B_w_gate.reshape(5, D // 5, F)
    wu = B_w_up.reshape(5, D // 5, F)
    like = lambda a: pltpu.VMEM(a.shape, a.dtype)
    return pl.pallas_call(
        _kernel,
        out_shape=jax.ShapeDtypeStruct(A_x.shape, A_x.dtype),
        in_specs=[pl.BlockSpec(memory_space=pl.ANY)] * 9,
        scratch_shapes=[
            like(A_x), like(B_w_r), like(wq), like(wo), like(wg), like(wu), like(B_w_down),
            pltpu.VMEM((NBUF, Dh, W), A_k_cache.dtype),
            pltpu.VMEM((NBUF, Dh, W), A_v_cache.dtype),
            pltpu.VMEM((H, 8, Dh), jnp.bfloat16),
            pltpu.VMEM((H, 8, Dh), jnp.bfloat16),
            pltpu.VMEM((8, W), jnp.bfloat16),
            pltpu.VMEM((8, 128), jnp.float32),
            pltpu.SemaphoreType.DMA((NBUF,)), pltpu.SemaphoreType.DMA((NBUF,)),
            pltpu.SemaphoreType.DMA((6,)), pltpu.SemaphoreType.DMA((len(DOWN_EDGES) - 1,)),
        ],
        compiler_params=pltpu.CompilerParams(
            vmem_limit_bytes=100 * 2**20,
            disable_bounds_checks=True, disable_semaphore_checks=True),
    )(A_x, kt, vt, wq, wo, B_w_r, wg, wu, B_w_down)
```

```python
from functools import partial

import jax
import jax.numpy as jnp
from jax import lax
import jax.experimental.pallas as pl
import jax.experimental.pallas.tpu as pltpu

EPS = 1e-5
LEAD = 26
WARMUP = 6
KV_ROWS, KV_COLS = 32, 512
NBUF = 4
WQ_SPLIT, WO_SPLIT, GU_SPLIT = 5, 3, 4
DOWN_ROWS = 32
TAIL = 256
TAIL_ROWS, TAIL_GROUP = 8, 32


def _layernorm(x):
    m = jnp.mean(x, axis=-1, keepdims=True)
    d = x - m
    v = jnp.mean(d * d, axis=-1, keepdims=True)
    return d / jnp.sqrt(v + EPS)


def _divmod(n, d, limit):
    m = -(-(1 << 16) // d)
    assert all((i * m) >> 16 == i // d for i in range(limit))
    q = (n * m) >> 16
    return q, n - q * d


class _Stream:
    def __init__(self, low, high):
        self.todo = {1: list(low), 0: list(high)}

    def start(self, steps=1 << 30, queues=(1, 0)):
        while steps > 0:
            live = [q for q in queues if self.todo[q]]
            if not live:
                return
            heads = {q: self.todo[q][0] for q in live}
            k = min([steps] + [end - first for _, first, end in heads.values()])

            def body(n, _, live=live, heads=heads):
                for q in live:
                    heads[q][0](heads[q][1] + n).start(priority=q)
            lax.fori_loop(0, k, body, None)
            for q in live:
                copy, first, end = heads[q]
                if first + k < end:
                    self.todo[q][0] = (copy, first + k, end)
                else:
                    self.todo[q].pop(0)
            steps -= k


def _kernel(x_hbm, kt_hbm, vt_hbm, wq_hbm, wo_hbm, wr_hbm, wg_hbm, wu_hbm, wd_hbm,
            o_ref,
            x_s, wr_s, wq_s, wo_s, wg_s, wu_s, wd_s, k_s, v_s, q_s, oh_s, p_s, l_s, c_s,
            sem_k, sem_v, sem_w, sem_d):
    _, H, Dh, Sk = kt_hbm.shape
    W = k_s.shape[-1]
    D = x_hbm.shape[-1]
    F = wd_hbm.shape[0]
    f32, bf16 = jnp.float32, jnp.bfloat16

    def span(start, size):
        return pl.ds(pl.multiple_of(start * size, size), size)

    per_col = Dh // KV_ROWS // 2
    n_kv = per_col * (W // KV_COLS)

    def kv_copy(which, h, odd, n):
        src, dst, sem = ((kt_hbm, k_s, sem_k), (vt_hbm, v_s, sem_v))[which]
        c, i = _divmod(n, per_col, n_kv)
        rows, slot = span(2 * i + odd, KV_ROWS), h & (NBUF - 1)
        return pltpu.make_async_copy(
            src.at[0, h, rows, span((Sk - W) // KV_COLS + c, KV_COLS)],
            dst.at[slot, rows, span(c, KV_COLS)], sem.at[slot])

    n_wq = 192

    def wq_copy(odd, n):
        a, b = _divmod(n, 3, n_wq)
        r, c = _divmod(b * 64 + a, 12, n_wq)
        idx = (pl.ds(2, 3) if odd else pl.ds(0, 2), span(r, 8), span(c, 512))
        return pltpu.make_async_copy(wq_hbm.at[idx], wq_s.at[idx], sem_w.at[0])

    n_wo = 128

    def wo_copy(odd, n):
        a, b = _divmod(2 * n + odd, 5, 2 * n_wo)
        r = jnp.where(a == 51, 255, b * 51 + a)
        idx = (slice(None), span(r, 8), slice(None))
        return pltpu.make_async_copy(wo_hbm.at[idx], wo_s.at[idx], sem_w.at[1])

    n_gu = 60

    def gu_copy(odd, n):
        src, dst = ((wg_hbm, wg_s), (wu_hbm, wu_s))[odd]
        r, c = _divmod(n, 3, n_gu)
        idx = (slice(None), span(r, 8), span(c, 512))
        return pltpu.make_async_copy(src.at[idx], dst.at[idx], sem_w.at[2])

    half = (F - TAIL) // 2
    cut = half * 3 // 5 // 128 * 128
    n_wd = half // DOWN_ROWS

    def wd_copy(odd, n):
        idx = (span(odd * n_wd + n, DOWN_ROWS), slice(None))
        part = jnp.where(n * DOWN_ROWS >= cut, 1, 0)
        return pltpu.make_async_copy(wd_hbm.at[idx], wd_s.at[idx], sem_d.at[part])

    def tail_copy(n):
        idx = (span(2 * half // TAIL_ROWS + n, TAIL_ROWS), slice(None))
        group = _divmod(n, TAIL_GROUP // TAIL_ROWS, TAIL // TAIL_ROWS)[0]
        return pltpu.make_async_copy(wd_hbm.at[idx], wd_s.at[idx], sem_d.at[2 + group])

    def kv_run(h, odd, first, end):
        run = []
        while first < end:
            b, n = divmod(first, n_kv)
            k = min(n_kv - n, end - first)
            run.append((partial(kv_copy, b % 2, h + b // 2, odd), n, n + k))
            first += k
        return run

    def landed(dst, sem):
        pltpu.make_async_copy(dst, dst, sem).wait()

    def q_proj(g0, g1):
        def body(g, _):
            w = wq_s[:, :, span(g, 4 * Dh)].reshape(D, 4 * Dh)
            q = jnp.dot(xn, w, preferred_element_type=f32)
            for j in range(4):
                q_s[g * 4 + j] = q[:, j * Dh:(j + 1) * Dh].astype(bf16)
        lax.fori_loop(g0, g1, body, None)

    def scores(h):
        slot = h & (NBUF - 1)
        landed(k_s.at[slot], sem_k.at[slot])
        s = jnp.dot(q_s[h], k_s[slot], preferred_element_type=f32) * Dh ** -0.5
        e = jnp.exp(s - jnp.max(s, axis=-1, keepdims=True))
        l_s[...] = jnp.broadcast_to(jnp.sum(e, axis=-1, keepdims=True), l_s.shape)
        p_s[...] = e.astype(bf16)

    def values(h):
        slot = h & (NBUF - 1)
        landed(v_s.at[slot], sem_v.at[slot])
        a = lax.dot_general(p_s[...], v_s[slot], (((1,), (1,)), ((), ())),
                            preferred_element_type=f32)
        oh_s[h] = (a / l_s[:, :1]).astype(bf16)

    def o_proj(g0, g1, y):
        wo_rows = wo_s.reshape(H * Dh, D)

        def body(g, y):
            for j in range(4):
                h = g * 4 + j
                y = y + jnp.dot(oh_s[h], wo_rows[span(h, Dh), :], preferred_element_type=f32)
            return y
        return lax.fori_loop(g0, g1, body, y)

    x_copy = pltpu.make_async_copy(x_hbm, x_s, sem_w.at[3])
    wr_copy = pltpu.make_async_copy(wr_hbm, wr_s, sem_w.at[4])

    stream = _Stream([(partial(wq_copy, 0), 0, n_wq)] + kv_run(0, 0, 0, LEAD),
                     [(partial(wq_copy, 1), 0, n_wq)])
    stream.start(WARMUP)
    stream.start(LEAD, queues=(1,))
    x_copy.start()
    wr_copy.start()
    stream.start()

    x_copy.wait()
    wr_copy.wait()
    x = x_s[0].astype(f32)
    xn = jnp.broadcast_to(_layernorm(x), (8, D)).astype(bf16)

    def head_round(j, _):
        stream = _Stream(kv_run(j, 0, LEAD, LEAD + 2 * n_kv), kv_run(j, 1, 0, 2 * n_kv))
        stream.start(n_kv)
        pl.when(j == 1)(lambda: q_proj(4, 8))
        pl.when(j >= 2)(lambda: values(j - 2))
        stream.start()

        @pl.when(j == 0)
        def _():
            landed(wq_s, sem_w.at[0])
            q_proj(0, 4)
        pl.when(j >= 1)(lambda: scores(j - 1))
    lax.fori_loop(0, H - 1, head_round, None)

    def rest(odd):
        return [(partial(wo_copy, odd), 0, n_wo), (partial(gu_copy, odd), 0, n_gu),
                (partial(wd_copy, odd), 0, n_wd)]

    stream = _Stream(kv_run(H - 1, 0, LEAD, 2 * n_kv) + rest(0) + [(tail_copy, 0, TAIL // TAIL_ROWS)],
                     kv_run(H - 1, 1, 0, 2 * n_kv) + rest(1))
    for work, h in ((values, H - 3), (scores, H - 2), (values, H - 2), (scores, H - 1), (values, H - 1)):
        stream.start(n_kv)
        work(h)
    stream.start(n_wo - 3 * n_kv + 32)

    landed(wo_s, sem_w.at[1])
    y = jnp.zeros((8, D), f32)
    for g in range(0, H // 4, 2):
        y = o_proj(g, g + 2, y)
        stream.start((n_gu + n_wd - 32) // 3 + 1)
    stream.start()

    hres = x + y[0:1, :]
    hn = _layernorm(hres)
    wr = wr_s[...].astype(f32).reshape(1, D)
    gate = jax.nn.sigmoid(jnp.sum(hn * wr, axis=-1, keepdims=True))
    hb = jnp.broadcast_to(hn, (8, D)).astype(bf16)

    landed(wg_s, sem_w.at[2])
    landed(wu_s, sem_w.at[2])
    g = jnp.dot(hb, wg_s[...].reshape(D, F), preferred_element_type=f32)
    u = jnp.dot(hb, wu_s[...].reshape(D, F), preferred_element_type=f32)
    gu = g * jax.nn.sigmoid(g) * u
    for r in range(0, TAIL, 128):
        c = gu[:1, 2 * half + r:2 * half + r + 128] * gate
        c_s[r:r + 128, :] = jnp.broadcast_to(c, (128, 128)).T
    gu = gu.astype(bf16)

    y = jnp.zeros((8, D), f32)
    for part, (r0, r1) in enumerate(((0, cut), (cut, half))):
        for o in (0, half):
            landed(wd_s.at[pl.ds(o + r0, r1 - r0)], sem_d.at[part])
        for o in (0, half):
            y = y + jnp.dot(gu[:, o + r0:o + r1], wd_s[o + r0:o + r1, :],
                            preferred_element_type=f32)
    base = hres + (hn + y[:1] * gate)

    acc = jnp.zeros((8, D), f32)
    for j, r in enumerate(range(0, TAIL, TAIL_GROUP)):
        landed(wd_s.at[pl.ds(2 * half + r, TAIL_GROUP)], sem_d.at[2 + j])
        w = wd_s[2 * half + r:2 * half + r + TAIL_GROUP, :].astype(f32)
        for t in range(0, TAIL_GROUP, 8):
            c = c_s[r + t:r + t + 8, :]
            acc = acc + w[t:t + 8, :] * jnp.concatenate([c] * (D // 128), axis=1)
    o_ref[0] = (base + jnp.sum(acc, axis=0, keepdims=True)).astype(o_ref.dtype)


@jax.jit
def pallas_sequential_preLN__sliding_block_cached__moe_arch_mod__decode_kernel(
    A_x: jax.Array,
    A_k_cache: jax.Array,
    A_v_cache: jax.Array,
    A_wq: jax.Array,
    A_wo: jax.Array,
    B_x: jax.Array,
    B_w_r: jax.Array,
    B_w_gate: jax.Array,
    B_w_up: jax.Array,
    B_w_down: jax.Array,
):
    del B_x
    _, H, Sk, Dh = A_k_cache.shape
    D = A_x.shape[-1]
    F = B_w_gate.shape[-1]
    W = min(4096, max(256, Sk // 4))
    kt = jnp.transpose(A_k_cache, (0, 1, 3, 2))
    vt = jnp.transpose(A_v_cache, (0, 1, 3, 2))
    wq = A_wq.reshape(WQ_SPLIT, D // WQ_SPLIT, H * Dh)
    wo = A_wo.reshape(WO_SPLIT, H * Dh // WO_SPLIT, D)
    wg = B_w_gate.reshape(GU_SPLIT, D // GU_SPLIT, F)
    wu = B_w_up.reshape(GU_SPLIT, D // GU_SPLIT, F)
    like = lambda a: pltpu.VMEM(a.shape, a.dtype)
    return pl.pallas_call(
        _kernel,
        out_shape=jax.ShapeDtypeStruct(A_x.shape, A_x.dtype),
        in_specs=[pl.BlockSpec(memory_space=pl.ANY)] * 9,
        scratch_shapes=[
            like(A_x), like(B_w_r), like(wq), like(wo), like(wg), like(wu), like(B_w_down),
            pltpu.VMEM((NBUF, Dh, W), A_k_cache.dtype),
            pltpu.VMEM((NBUF, Dh, W), A_v_cache.dtype),
            pltpu.VMEM((H, 8, Dh), jnp.bfloat16),
            pltpu.VMEM((H, 8, Dh), jnp.bfloat16),
            pltpu.VMEM((8, W), jnp.bfloat16),
            pltpu.VMEM((8, 128), jnp.float32),
            pltpu.VMEM((TAIL, 128), jnp.float32),
            pltpu.SemaphoreType.DMA((NBUF,)), pltpu.SemaphoreType.DMA((NBUF,)),
            pltpu.SemaphoreType.DMA((5,)), pltpu.SemaphoreType.DMA((2 + TAIL // TAIL_GROUP,)),
        ],
        compiler_params=pltpu.CompilerParams(
            vmem_limit_bytes=100 * 2**20,
            disable_bounds_checks=True, disable_semaphore_checks=True),
    )(A_x, kt, vt, wq, wo, B_w_r, wg, wu, B_w_down)
```

```python
from functools import partial

import jax
import jax.numpy as jnp
from jax import lax
import jax.experimental.pallas as pl
import jax.experimental.pallas.tpu as pltpu

EPS = 1e-5
LEAD = 26
WARMUP = 6
KV_ROWS, KV_COLS = 32, 512
NBUF = 4
WQ_SPLIT, WO_SPLIT, GU_SPLIT = 5, 3, 4
DOWN_ROWS = 32
TAIL = 256
TAIL_ROWS, TAIL_GROUP = 8, 32


def _layernorm(x):
    m = jnp.mean(x, axis=-1, keepdims=True)
    d = x - m
    v = jnp.mean(d * d, axis=-1, keepdims=True)
    return d / jnp.sqrt(v + EPS)


def _divmod(n, d, limit):
    m = -(-(1 << 16) // d)
    assert all((i * m) >> 16 == i // d for i in range(limit))
    q = (n * m) >> 16
    return q, n - q * d


class _Stream:
    def __init__(self, low, high):
        self.todo = {1: list(low), 0: list(high)}

    def start(self, steps=1 << 30, queues=(1, 0)):
        while steps > 0:
            live = [q for q in queues if self.todo[q]]
            if not live:
                return
            heads = {q: self.todo[q][0] for q in live}
            k = min([steps] + [end - first for _, first, end in heads.values()])

            def body(n, _, live=live, heads=heads):
                for q in live:
                    heads[q][0](heads[q][1] + n).start(priority=q)
            lax.fori_loop(0, k, body, None)
            for q in live:
                copy, first, end = heads[q]
                if first + k < end:
                    self.todo[q][0] = (copy, first + k, end)
                else:
                    self.todo[q].pop(0)
            steps -= k


def _kernel(x_hbm, kt_hbm, vt_hbm, wq_hbm, wo_hbm, wr_hbm, wg_hbm, wu_hbm, wd_hbm,
            o_ref,
            x_s, wr_s, wq_s, wo_s, wg_s, wu_s, wd_s, k_s, v_s, q_s, p_s, l_s, even_s, o_s, c_s,
            sem_k, sem_v, sem_w, sem_d):
    _, H, Dh, Sk = kt_hbm.shape
    W = k_s.shape[-1]
    D = x_hbm.shape[-1]
    F = wd_hbm.shape[0]
    f32, bf16 = jnp.float32, jnp.bfloat16

    def span(start, size):
        return pl.ds(pl.multiple_of(start * size, size), size)

    per_col = Dh // KV_ROWS // 2
    n_kv = per_col * (W // KV_COLS)

    def kv_copy(which, h, odd, n):
        src, dst, sem = ((kt_hbm, k_s, sem_k), (vt_hbm, v_s, sem_v))[which]
        c, i = _divmod(n, per_col, n_kv)
        rows, slot = span(2 * i + odd, KV_ROWS), h & (NBUF - 1)
        return pltpu.make_async_copy(
            src.at[0, h, rows, span((Sk - W) // KV_COLS + c, KV_COLS)],
            dst.at[slot, rows, span(c, KV_COLS)], sem.at[slot])

    n_wq = 192

    def wq_copy(odd, n):
        a, b = _divmod(n, 3, n_wq)
        r, c = _divmod(b * 64 + a, 12, n_wq)
        idx = (pl.ds(2, 3) if odd else pl.ds(0, 2), span(r, 8), span(c, 512))
        return pltpu.make_async_copy(wq_hbm.at[idx], wq_s.at[idx], sem_w.at[0])

    n_wo = 128

    def wo_copy(odd, n):
        a, b = _divmod(2 * n + odd, 5, 2 * n_wo)
        r = jnp.where(a == 51, 255, b * 51 + a)
        idx = (slice(None), span(r, 8), slice(None))
        return pltpu.make_async_copy(wo_hbm.at[idx], wo_s.at[idx], sem_w.at[1])

    n_gu = 60

    def gu_copy(odd, n):
        src, dst = ((wg_hbm, wg_s), (wu_hbm, wu_s))[odd]
        r, c = _divmod(n, 3, n_gu)
        idx = (slice(None), span(r, 8), span(c, 512))
        return pltpu.make_async_copy(src.at[idx], dst.at[idx], sem_w.at[2])

    half = (F - TAIL) // 2
    cut = half * 3 // 5 // 128 * 128
    n_wd = half // DOWN_ROWS

    def wd_copy(odd, n):
        idx = (span(odd * n_wd + n, DOWN_ROWS), slice(None))
        part = jnp.where(n * DOWN_ROWS >= cut, 1, 0)
        return pltpu.make_async_copy(wd_hbm.at[idx], wd_s.at[idx], sem_d.at[part])

    def tail_copy(n):
        idx = (span(2 * half // TAIL_ROWS + n, TAIL_ROWS), slice(None))
        group = _divmod(n, TAIL_GROUP // TAIL_ROWS, TAIL // TAIL_ROWS)[0]
        return pltpu.make_async_copy(wd_hbm.at[idx], wd_s.at[idx], sem_d.at[2 + group])

    def kv_run(h, odd, first, end):
        run = []
        while first < end:
            b, n = divmod(first, n_kv)
            k = min(n_kv - n, end - first)
            run.append((partial(kv_copy, b % 2, h + b // 2, odd), n, n + k))
            first += k
        return run

    def landed(dst, sem):
        pltpu.make_async_copy(dst, dst, sem).wait()

    def q_proj(g0, g1):
        def body(g, _):
            w = wq_s[:, :, span(g, 4 * Dh)].reshape(D, 4 * Dh)
            q = jnp.dot(xn, w, preferred_element_type=f32)
            for j in range(4):
                q_s[g * 4 + j] = q[:, j * Dh:(j + 1) * Dh].astype(bf16)
        lax.fori_loop(g0, g1, body, None)

    def scores(h):
        slot = h & (NBUF - 1)
        landed(k_s.at[slot], sem_k.at[slot])
        s = jnp.dot(q_s[h], k_s[slot], preferred_element_type=f32) * Dh ** -0.5
        e = jnp.exp(s - jnp.max(s, axis=-1, keepdims=True))
        l_s[...] = jnp.broadcast_to(jnp.sum(e, axis=-1, keepdims=True), l_s.shape)
        p_s[...] = e.astype(bf16)

    def values(h):
        slot = h & (NBUF - 1)
        landed(v_s.at[slot], sem_v.at[slot])
        a = lax.dot_general(p_s[...], v_s[slot], (((1,), (1,)), ((), ())),
                            preferred_element_type=f32)
        o = a / l_s[:, :1]

        @pl.when(h & 1 == 0)
        def _():
            even_s[...] = o

        @pl.when(h & 1 == 1)
        def _():
            o_s[:, span(h >> 1, 2 * Dh)] = jnp.concatenate([even_s[...], o], axis=1).astype(bf16)

    def o_proj(c0, c1, y):
        rows = wo_s.shape[1] // 2

        def body(c, y):
            return y + jnp.dot(o_s[:, span(c, rows)], wo_s[c >> 1, span(c & 1, rows), :],
                               preferred_element_type=f32)
        return lax.fori_loop(c0, c1, body, y)

    x_copy = pltpu.make_async_copy(x_hbm, x_s, sem_w.at[3])
    wr_copy = pltpu.make_async_copy(wr_hbm, wr_s, sem_w.at[4])

    stream = _Stream([(partial(wq_copy, 0), 0, n_wq)] + kv_run(0, 0, 0, LEAD),
                     [(partial(wq_copy, 1), 0, n_wq)])
    stream.start(WARMUP)
    stream.start(LEAD, queues=(1,))
    x_copy.start()
    wr_copy.start()
    stream.start()

    x_copy.wait()
    wr_copy.wait()
    x = x_s[0].astype(f32)
    xn = jnp.broadcast_to(_layernorm(x), (8, D)).astype(bf16)

    def head_round(j, _):
        stream = _Stream(kv_run(j, 0, LEAD, LEAD + 2 * n_kv), kv_run(j, 1, 0, 2 * n_kv))
        stream.start(n_kv)
        pl.when(j == 1)(lambda: q_proj(4, 8))
        pl.when(j >= 2)(lambda: values(j - 2))
        stream.start()

        @pl.when(j == 0)
        def _():
            landed(wq_s, sem_w.at[0])
            q_proj(0, 4)
        pl.when(j >= 1)(lambda: scores(j - 1))
    lax.fori_loop(0, H - 1, head_round, None)

    def rest(odd):
        return [(partial(wo_copy, odd), 0, n_wo), (partial(gu_copy, odd), 0, n_gu),
                (partial(wd_copy, odd), 0, n_wd)]

    stream = _Stream(kv_run(H - 1, 0, LEAD, 2 * n_kv) + rest(0) + [(tail_copy, 0, TAIL // TAIL_ROWS)],
                     kv_run(H - 1, 1, 0, 2 * n_kv) + rest(1))
    for work, h in ((values, H - 3), (scores, H - 2), (values, H - 2), (scores, H - 1), (values, H - 1)):
        stream.start(n_kv)
        work(h)
    stream.start(n_wo - 3 * n_kv + 32)

    landed(wo_s, sem_w.at[1])
    y = jnp.zeros((8, D), f32)
    for c in range(0, 2 * WO_SPLIT, 2):
        y = o_proj(c, c + 2, y)
        stream.start((n_gu + n_wd - 32) // 2 + 1)
    stream.start()

    hres = x + y[0:1, :]
    hn = _layernorm(hres)
    wr = wr_s[...].astype(f32).reshape(1, D)
    gate = jax.nn.sigmoid(jnp.sum(hn * wr, axis=-1, keepdims=True))
    hb = jnp.broadcast_to(hn, (8, D)).astype(bf16)

    landed(wg_s, sem_w.at[2])
    landed(wu_s, sem_w.at[2])
    g = jnp.dot(hb, wg_s[...].reshape(D, F), preferred_element_type=f32)
    u = jnp.dot(hb, wu_s[...].reshape(D, F), preferred_element_type=f32)
    gu = g * jax.nn.sigmoid(g) * u
    for r in range(0, TAIL, 128):
        c = gu[:1, 2 * half + r:2 * half + r + 128] * gate
        c_s[r:r + 128, :] = jnp.broadcast_to(c, (128, 128)).T
    gu = gu.astype(bf16)

    y = jnp.zeros((8, D), f32)
    for part, (r0, r1) in enumerate(((0, cut), (cut, half))):
        for o in (0, half):
            landed(wd_s.at[pl.ds(o + r0, r1 - r0)], sem_d.at[part])
        for o in (0, half):
            y = y + jnp.dot(gu[:, o + r0:o + r1], wd_s[o + r0:o + r1, :],
                            preferred_element_type=f32)
    base = hres + (hn + y[:1] * gate)

    acc = jnp.zeros((8, D), f32)
    for j, r in enumerate(range(0, TAIL, TAIL_GROUP)):
        landed(wd_s.at[pl.ds(2 * half + r, TAIL_GROUP)], sem_d.at[2 + j])
        w = wd_s[2 * half + r:2 * half + r + TAIL_GROUP, :].astype(f32)
        for t in range(0, TAIL_GROUP, 8):
            c = c_s[r + t:r + t + 8, :]
            acc = acc + w[t:t + 8, :] * jnp.concatenate([c] * (D // 128), axis=1)
    o_ref[0] = (base + jnp.sum(acc, axis=0, keepdims=True)).astype(o_ref.dtype)


@jax.jit
def pallas_sequential_preLN__sliding_block_cached__moe_arch_mod__decode_kernel(
    A_x: jax.Array,
    A_k_cache: jax.Array,
    A_v_cache: jax.Array,
    A_wq: jax.Array,
    A_wo: jax.Array,
    B_x: jax.Array,
    B_w_r: jax.Array,
    B_w_gate: jax.Array,
    B_w_up: jax.Array,
    B_w_down: jax.Array,
):
    del B_x
    _, H, Sk, Dh = A_k_cache.shape
    D = A_x.shape[-1]
    F = B_w_gate.shape[-1]
    W = min(4096, max(256, Sk // 4))
    kt = jnp.transpose(A_k_cache, (0, 1, 3, 2))
    vt = jnp.transpose(A_v_cache, (0, 1, 3, 2))
    wq = A_wq.reshape(WQ_SPLIT, D // WQ_SPLIT, H * Dh)
    wo = A_wo.reshape(WO_SPLIT, H * Dh // WO_SPLIT, D)
    wg = B_w_gate.reshape(GU_SPLIT, D // GU_SPLIT, F)
    wu = B_w_up.reshape(GU_SPLIT, D // GU_SPLIT, F)
    like = lambda a: pltpu.VMEM(a.shape, a.dtype)
    return pl.pallas_call(
        _kernel,
        out_shape=jax.ShapeDtypeStruct(A_x.shape, A_x.dtype),
        in_specs=[pl.BlockSpec(memory_space=pl.ANY)] * 9,
        scratch_shapes=[
            like(A_x), like(B_w_r), like(wq), like(wo), like(wg), like(wu), like(B_w_down),
            pltpu.VMEM((NBUF, Dh, W), A_k_cache.dtype),
            pltpu.VMEM((NBUF, Dh, W), A_v_cache.dtype),
            pltpu.VMEM((H, 8, Dh), jnp.bfloat16),
            pltpu.VMEM((8, W), jnp.bfloat16),
            pltpu.VMEM((8, 128), jnp.float32),
            pltpu.VMEM((8, Dh), jnp.float32),
            pltpu.VMEM((8, H * Dh), jnp.bfloat16),
            pltpu.VMEM((TAIL, 128), jnp.float32),
            pltpu.SemaphoreType.DMA((NBUF,)), pltpu.SemaphoreType.DMA((NBUF,)),
            pltpu.SemaphoreType.DMA((5,)), pltpu.SemaphoreType.DMA((2 + TAIL // TAIL_GROUP,)),
        ],
        compiler_params=pltpu.CompilerParams(
            vmem_limit_bytes=100 * 2**20,
            disable_bounds_checks=True, disable_semaphore_checks=True),
    )(A_x, kt, vt, wq, wo, B_w_r, wg, wu, B_w_down)
```

```python
from functools import partial

import jax
import jax.numpy as jnp
from jax import lax
import jax.experimental.pallas as pl
import jax.experimental.pallas.tpu as pltpu

EPS = 1e-5
LEAD = 26
WARMUP = 6
KV_ROWS, KV_COLS = 32, 512
NBUF = 4
WQ_SPLIT, WO_SPLIT, GU_SPLIT = 5, 3, 4
DOWN_ROWS = 32
TAIL = 256
TAIL_ROWS, TAIL_GROUP = 8, 16


def _layernorm(x):
    m = jnp.mean(x, axis=-1, keepdims=True)
    d = x - m
    v = jnp.mean(d * d, axis=-1, keepdims=True)
    return d / jnp.sqrt(v + EPS)


def _divmod(n, d, limit):
    m = -(-(1 << 16) // d)
    assert all((i * m) >> 16 == i // d for i in range(limit))
    q = (n * m) >> 16
    return q, n - q * d


class _Stream:
    def __init__(self, low, high):
        self.todo = {1: list(low), 0: list(high)}

    def start(self, steps=1 << 30, queues=(1, 0)):
        while steps > 0:
            live = [q for q in queues if self.todo[q]]
            if not live:
                return
            heads = {q: self.todo[q][0] for q in live}
            k = min([steps] + [end - first for _, first, end in heads.values()])

            def body(n, _, live=live, heads=heads):
                for q in live:
                    heads[q][0](heads[q][1] + n).start(priority=q)
            lax.fori_loop(0, k, body, None)
            for q in live:
                copy, first, end = heads[q]
                if first + k < end:
                    self.todo[q][0] = (copy, first + k, end)
                else:
                    self.todo[q].pop(0)
            steps -= k


def _kernel(x_hbm, kt_hbm, vt_hbm, wq_hbm, wo_hbm, wr_hbm, wg_hbm, wu_hbm, wd_hbm,
            o_ref,
            x_s, wr_s, wq_s, wo_s, wg_s, wu_s, wd_s, k_s, v_s, q_s, p_s, l_s, even_s, o_s, c_s,
            sem_k, sem_v, sem_w, sem_d):
    _, H, Dh, Sk = kt_hbm.shape
    W = k_s.shape[-1]
    D = x_hbm.shape[-1]
    F = wd_hbm.shape[0]
    f32, bf16 = jnp.float32, jnp.bfloat16

    def span(start, size):
        return pl.ds(pl.multiple_of(start * size, size), size)

    per_col = Dh // KV_ROWS // 2
    n_kv = per_col * (W // KV_COLS)

    def kv_copy(which, h, odd, n):
        src, dst, sem = ((kt_hbm, k_s, sem_k), (vt_hbm, v_s, sem_v))[which]
        c, i = _divmod(n, per_col, n_kv)
        rows, slot = span(2 * i + odd, KV_ROWS), h & (NBUF - 1)
        return pltpu.make_async_copy(
            src.at[0, h, rows, span((Sk - W) // KV_COLS + c, KV_COLS)],
            dst.at[slot, rows, span(c, KV_COLS)], sem.at[slot])

    n_wq = 192

    def wq_copy(odd, n):
        a, b = _divmod(n, 3, n_wq)
        r, c = _divmod(b * 64 + a, 12, n_wq)
        idx = (pl.ds(4, 1) if odd else pl.ds(0, 4), span(r, 8), span(c, 512))
        return pltpu.make_async_copy(wq_hbm.at[idx], wq_s.at[idx], sem_w.at[0])

    n_wo = 128

    def wo_copy(odd, n):
        a, b = _divmod(2 * n + odd, 5, 2 * n_wo)
        r = jnp.where(a == 51, 153, b * 51 + a + jnp.where(b >= 3, 1, 0))
        idx = (slice(None), span(r, 8), slice(None))
        return pltpu.make_async_copy(wo_hbm.at[idx], wo_s.at[idx], sem_w.at[1])

    n_gu = 60

    def gu_copy(odd, n):
        src, dst = ((wg_hbm, wg_s), (wu_hbm, wu_s))[odd]
        r, c = _divmod(n, 3, n_gu)
        idx = (slice(None), span(r, 8), span(c, 512))
        return pltpu.make_async_copy(src.at[idx], dst.at[idx], sem_w.at[2])

    half = (F - TAIL) // 2
    cut = half - 128
    n_wd = half // DOWN_ROWS

    def wd_copy(odd, n):
        idx = (span(odd * n_wd + n, DOWN_ROWS), slice(None))
        part = jnp.where(n * DOWN_ROWS >= cut, 1, 0)
        return pltpu.make_async_copy(wd_hbm.at[idx], wd_s.at[idx], sem_d.at[part])

    def tail_copy(n):
        idx = (span(2 * half // TAIL_ROWS + n, TAIL_ROWS), slice(None))
        group = _divmod(n, TAIL_GROUP // TAIL_ROWS, TAIL // TAIL_ROWS)[0]
        return pltpu.make_async_copy(wd_hbm.at[idx], wd_s.at[idx], sem_d.at[2 + group])

    def kv_run(h, odd, first, end):
        run = []
        while first < end:
            b, n = divmod(first, n_kv)
            k = min(n_kv - n, end - first)
            run.append((partial(kv_copy, b % 2, h + b // 2, odd), n, n + k))
            first += k
        return run

    def landed(dst, sem):
        pltpu.make_async_copy(dst, dst, sem).wait()

    def q_proj(g0, g1):
        def body(g, _):
            w = wq_s[:, :, span(g, 4 * Dh)].reshape(D, 4 * Dh)
            q = jnp.dot(xn, w, preferred_element_type=f32)
            for j in range(4):
                q_s[g * 4 + j] = q[:, j * Dh:(j + 1) * Dh].astype(bf16)
        lax.fori_loop(g0, g1, body, None)

    def scores(h):
        slot = h & (NBUF - 1)
        landed(k_s.at[slot], sem_k.at[slot])
        s = jnp.dot(q_s[h], k_s[slot], preferred_element_type=f32) * Dh ** -0.5
        e = jnp.exp(s - jnp.max(s, axis=-1, keepdims=True))
        l_s[...] = jnp.broadcast_to(jnp.sum(e, axis=-1, keepdims=True), l_s.shape)
        p_s[...] = e.astype(bf16)

    def values(h):
        slot = h & (NBUF - 1)
        landed(v_s.at[slot], sem_v.at[slot])
        a = lax.dot_general(p_s[...], v_s[slot], (((1,), (1,)), ((), ())),
                            preferred_element_type=f32)
        o = a / l_s[:, :1]

        @pl.when(h & 1 == 0)
        def _():
            even_s[...] = o

        @pl.when(h & 1 == 1)
        def _():
            o_s[:, span(h >> 1, 2 * Dh)] = jnp.concatenate([even_s[...], o], axis=1).astype(bf16)

    def o_proj(c0, c1, y):
        rows = wo_s.shape[1] // 2

        def body(c, y):
            return y + jnp.dot(o_s[:, span(c, rows)], wo_s[c >> 1, span(c & 1, rows), :],
                               preferred_element_type=f32)
        return lax.fori_loop(c0, c1, body, y)

    x_copy = pltpu.make_async_copy(x_hbm, x_s, sem_w.at[3])
    wr_copy = pltpu.make_async_copy(wr_hbm, wr_s, sem_w.at[4])

    stream = _Stream([(partial(wq_copy, 0), 0, n_wq)] + kv_run(0, 0, 0, LEAD),
                     [(partial(wq_copy, 1), 0, n_wq)])
    stream.start(WARMUP)
    stream.start(LEAD, queues=(1,))
    x_copy.start()
    wr_copy.start()
    stream.start()

    x_copy.wait()
    wr_copy.wait()
    x = x_s[0].astype(f32)
    xn = jnp.broadcast_to(_layernorm(x), (8, D)).astype(bf16)

    def head_round(j, _):
        stream = _Stream(kv_run(j, 0, LEAD, LEAD + 2 * n_kv), kv_run(j, 1, 0, 2 * n_kv))
        stream.start(n_kv)
        pl.when(j == 1)(lambda: q_proj(4, 8))
        pl.when(j >= 2)(lambda: values(j - 2))
        stream.start()

        @pl.when(j == 0)
        def _():
            landed(wq_s, sem_w.at[0])
            q_proj(0, 4)
        pl.when(j >= 1)(lambda: scores(j - 1))
    lax.fori_loop(0, H - 1, head_round, None)

    def rest(odd):
        return [(partial(wo_copy, odd), 0, n_wo), (partial(gu_copy, odd), 0, n_gu),
                (partial(wd_copy, odd), 0, n_wd)]

    stream = _Stream(kv_run(H - 1, 0, LEAD, 2 * n_kv) + rest(0) + [(tail_copy, 0, TAIL // TAIL_ROWS)],
                     kv_run(H - 1, 1, 0, 2 * n_kv) + rest(1))
    for work, h in ((values, H - 3), (scores, H - 2), (values, H - 2), (scores, H - 1), (values, H - 1)):
        stream.start(n_kv)
        work(h)
    stream.start(n_wo - 3 * n_kv + 32)

    landed(wo_s, sem_w.at[1])
    y = jnp.zeros((8, D), f32)
    for c in range(0, 2 * WO_SPLIT, 2):
        y = o_proj(c, c + 2, y)
        stream.start((n_gu + n_wd - 32) // 2 + 1)
    stream.start()

    hres = x + y[0:1, :]
    hn = _layernorm(hres)
    wr = wr_s[...].astype(f32).reshape(1, D)
    gate = jax.nn.sigmoid(jnp.sum(hn * wr, axis=-1, keepdims=True))
    hb = jnp.broadcast_to(hn, (8, D)).astype(bf16)

    landed(wg_s, sem_w.at[2])
    landed(wu_s, sem_w.at[2])
    g = jnp.dot(hb, wg_s[...].reshape(D, F), preferred_element_type=f32)
    u = jnp.dot(hb, wu_s[...].reshape(D, F), preferred_element_type=f32)
    gu = g * jax.nn.sigmoid(g) * u
    for r in range(0, TAIL, 128):
        c = gu[:1, 2 * half + r:2 * half + r + 128] * gate
        c_s[r:r + 128, :] = jnp.broadcast_to(c, (128, 128)).T
    gu = gu.astype(bf16)

    y = jnp.zeros((8, D), f32)
    for part, (r0, r1) in enumerate(((0, cut), (cut, half))):
        for o in (0, half):
            landed(wd_s.at[pl.ds(o + r0, r1 - r0)], sem_d.at[part])
        for o in (0, half):
            y = y + jnp.dot(gu[:, o + r0:o + r1], wd_s[o + r0:o + r1, :],
                            preferred_element_type=f32)
    base = hres + (hn + y[:1] * gate)

    acc = jnp.zeros((8, D), f32)
    for j, r in enumerate(range(0, TAIL, TAIL_GROUP)):
        landed(wd_s.at[pl.ds(2 * half + r, TAIL_GROUP)], sem_d.at[2 + j])
        w = wd_s[2 * half + r:2 * half + r + TAIL_GROUP, :].astype(f32)
        for t in range(0, TAIL_GROUP, 8):
            c = c_s[r + t:r + t + 8, :]
            acc = acc + w[t:t + 8, :] * jnp.concatenate([c] * (D // 128), axis=1)
    o_ref[0] = (base + jnp.sum(acc, axis=0, keepdims=True)).astype(o_ref.dtype)


@jax.jit
def pallas_sequential_preLN__sliding_block_cached__moe_arch_mod__decode_kernel(
    A_x: jax.Array,
    A_k_cache: jax.Array,
    A_v_cache: jax.Array,
    A_wq: jax.Array,
    A_wo: jax.Array,
    B_x: jax.Array,
    B_w_r: jax.Array,
    B_w_gate: jax.Array,
    B_w_up: jax.Array,
    B_w_down: jax.Array,
):
    del B_x
    _, H, Sk, Dh = A_k_cache.shape
    D = A_x.shape[-1]
    F = B_w_gate.shape[-1]
    W = min(4096, max(256, Sk // 4))
    kt = jnp.transpose(A_k_cache, (0, 1, 3, 2))
    vt = jnp.transpose(A_v_cache, (0, 1, 3, 2))
    wq = A_wq.reshape(WQ_SPLIT, D // WQ_SPLIT, H * Dh)
    wo = A_wo.reshape(WO_SPLIT, H * Dh // WO_SPLIT, D)
    wg = B_w_gate.reshape(GU_SPLIT, D // GU_SPLIT, F)
    wu = B_w_up.reshape(GU_SPLIT, D // GU_SPLIT, F)
    like = lambda a: pltpu.VMEM(a.shape, a.dtype)
    return pl.pallas_call(
        _kernel,
        out_shape=jax.ShapeDtypeStruct(A_x.shape, A_x.dtype),
        in_specs=[pl.BlockSpec(memory_space=pl.ANY)] * 9,
        scratch_shapes=[
            like(A_x), like(B_w_r), like(wq), like(wo), like(wg), like(wu), like(B_w_down),
            pltpu.VMEM((NBUF, Dh, W), A_k_cache.dtype),
            pltpu.VMEM((NBUF, Dh, W), A_v_cache.dtype),
            pltpu.VMEM((H, 8, Dh), jnp.bfloat16),
            pltpu.VMEM((8, W), jnp.bfloat16),
            pltpu.VMEM((8, 128), jnp.float32),
            pltpu.VMEM((8, Dh), jnp.float32),
            pltpu.VMEM((8, H * Dh), jnp.bfloat16),
            pltpu.VMEM((TAIL, 128), jnp.float32),
            pltpu.SemaphoreType.DMA((NBUF,)), pltpu.SemaphoreType.DMA((NBUF,)),
            pltpu.SemaphoreType.DMA((5,)), pltpu.SemaphoreType.DMA((2 + TAIL // TAIL_GROUP,)),
        ],
        compiler_params=pltpu.CompilerParams(
            vmem_limit_bytes=100 * 2**20,
            disable_bounds_checks=True, disable_semaphore_checks=True),
    )(A_x, kt, vt, wq, wo, B_w_r, wg, wu, B_w_down)
```

```python
from functools import partial

import jax
import jax.numpy as jnp
from jax import lax
import jax.experimental.pallas as pl
import jax.experimental.pallas.tpu as pltpu

EPS = 1e-5
LEAD = 26
WARMUP = 6
KV_ROWS, KV_COLS = 32, 512
NBUF = 4
WQ_SPLIT, WO_SPLIT, GU_SPLIT = 5, 3, 4
DOWN_ROWS = 32
TAIL = 256
TAIL_ROWS, TAIL_GROUP = 8, 16


def _layernorm(x):
    m = jnp.mean(x, axis=-1, keepdims=True)
    d = x - m
    v = jnp.mean(d * d, axis=-1, keepdims=True)
    return d / jnp.sqrt(v + EPS)


def _divmod(n, d, limit):
    m = -(-(1 << 16) // d)
    assert all((i * m) >> 16 == i // d for i in range(limit))
    q = (n * m) >> 16
    return q, n - q * d


class _Stream:
    def __init__(self, low, high):
        self.todo = {1: list(low), 0: list(high)}

    def start(self, steps=1 << 30, queues=(1, 0)):
        while steps > 0:
            live = [q for q in queues if self.todo[q]]
            if not live:
                return
            heads = {q: self.todo[q][0] for q in live}
            k = min([steps] + [end - first for _, first, end in heads.values()])

            def body(n, _, live=live, heads=heads):
                for q in live:
                    heads[q][0](heads[q][1] + n).start(priority=q)
            lax.fori_loop(0, k, body, None)
            for q in live:
                copy, first, end = heads[q]
                if first + k < end:
                    self.todo[q][0] = (copy, first + k, end)
                else:
                    self.todo[q].pop(0)
            steps -= k


def _kernel(x_hbm, kt_hbm, vt_hbm, wq_hbm, wo_hbm, wr_hbm, wg_hbm, wu_hbm, wd_hbm,
            o_ref,
            x_s, wr_s, wq_s, wo_s, wg_s, wu_s, wd_s, k_s, v_s, q_s, p_s, l_s, even_s, o_s, c_s,
            sem_k, sem_v, sem_w, sem_d, sem_t):
    _, H, Dh, Sk = kt_hbm.shape
    W = k_s.shape[-1]
    D = x_hbm.shape[-1]
    F = wd_hbm.shape[0]
    f32, bf16 = jnp.float32, jnp.bfloat16

    def span(start, size):
        return pl.ds(pl.multiple_of(start * size, size), size)

    per_col = Dh // KV_ROWS // 2
    n_kv = per_col * (W // KV_COLS)

    def kv_copy(which, h, odd, n):
        src, dst, sem = ((kt_hbm, k_s, sem_k), (vt_hbm, v_s, sem_v))[which]
        c, i = _divmod(n, per_col, n_kv)
        rows, slot = span(2 * i + odd, KV_ROWS), h & (NBUF - 1)
        return pltpu.make_async_copy(
            src.at[0, h, rows, span((Sk - W) // KV_COLS + c, KV_COLS)],
            dst.at[slot, rows, span(c, KV_COLS)], sem.at[slot])

    n_wq = 192

    def wq_copy(odd, n):
        a, b = _divmod(n, 3, n_wq)
        r, c = _divmod(b * 64 + a, 12, n_wq)
        idx = (pl.ds(4, 1) if odd else pl.ds(0, 4), span(r, 8), span(c, 512))
        return pltpu.make_async_copy(wq_hbm.at[idx], wq_s.at[idx], sem_w.at[0])

    n_wo = 128

    def wo_copy(odd, n):
        a, b = _divmod(2 * n + odd, 5, 2 * n_wo)
        r = jnp.where(a == 51, 153, b * 51 + a + jnp.where(b >= 3, 1, 0))
        idx = (slice(None), span(r, 8), slice(None))
        return pltpu.make_async_copy(wo_hbm.at[idx], wo_s.at[idx], sem_w.at[1])

    n_gu = 60

    def gu_copy(odd, n):
        src, dst = ((wg_hbm, wg_s), (wu_hbm, wu_s))[odd]
        r, c = _divmod(n, 3, n_gu)
        idx = (slice(None), span(r, 8), span(c, 512))
        return pltpu.make_async_copy(src.at[idx], dst.at[idx], sem_w.at[2 + odd])

    half = (F - TAIL) // 2
    cut = half - 128
    n_wd = half // DOWN_ROWS

    def wd_copy(odd, n):
        idx = (span(odd * n_wd + n, DOWN_ROWS), slice(None))
        part = jnp.where(n * DOWN_ROWS >= cut, 1, 0)
        return pltpu.make_async_copy(wd_hbm.at[idx], wd_s.at[idx], sem_d.at[2 * odd + part])

    def tail_copy(n):
        idx = (span(2 * half // TAIL_ROWS + n, TAIL_ROWS), slice(None))
        group = _divmod(n, TAIL_GROUP // TAIL_ROWS, TAIL // TAIL_ROWS)[0]
        return pltpu.make_async_copy(wd_hbm.at[idx], wd_s.at[idx], sem_t.at[group])

    def kv_run(h, odd, first, end):
        run = []
        while first < end:
            b, n = divmod(first, n_kv)
            k = min(n_kv - n, end - first)
            run.append((partial(kv_copy, b % 2, h + b // 2, odd), n, n + k))
            first += k
        return run

    def landed(dst, sem):
        pltpu.make_async_copy(dst, dst, sem).wait()

    def q_proj(g0, g1):
        def body(g, _):
            w = wq_s[:, :, span(g, 4 * Dh)].reshape(D, 4 * Dh)
            q = jnp.dot(xn, w, preferred_element_type=f32)
            for j in range(4):
                q_s[g * 4 + j] = q[:, j * Dh:(j + 1) * Dh].astype(bf16)
        lax.fori_loop(g0, g1, body, None)

    def scores(h):
        slot = h & (NBUF - 1)
        landed(k_s.at[slot], sem_k.at[slot])
        s = jnp.dot(q_s[h], k_s[slot], preferred_element_type=f32) * Dh ** -0.5
        e = jnp.exp(s - jnp.max(s, axis=-1, keepdims=True))
        l_s[...] = jnp.broadcast_to(jnp.sum(e, axis=-1, keepdims=True), l_s.shape)
        p_s[...] = e.astype(bf16)

    def values(h):
        slot = h & (NBUF - 1)
        landed(v_s.at[slot], sem_v.at[slot])
        a = lax.dot_general(p_s[...], v_s[slot], (((1,), (1,)), ((), ())),
                            preferred_element_type=f32)
        o = a / l_s[:, :1]

        @pl.when(h & 1 == 0)
        def _():
            even_s[...] = o

        @pl.when(h & 1 == 1)
        def _():
            o_s[:, span(h >> 1, 2 * Dh)] = jnp.concatenate([even_s[...], o], axis=1).astype(bf16)

    def o_proj(c0, c1, y):
        rows = wo_s.shape[1] // 2

        def body(c, y):
            return y + jnp.dot(o_s[:, span(c, rows)], wo_s[c >> 1, span(c & 1, rows), :],
                               preferred_element_type=f32)
        return lax.fori_loop(c0, c1, body, y)

    x_copy = pltpu.make_async_copy(x_hbm, x_s, sem_w.at[4])
    wr_copy = pltpu.make_async_copy(wr_hbm, wr_s, sem_w.at[5])

    stream = _Stream([(partial(wq_copy, 0), 0, n_wq)] + kv_run(0, 0, 0, LEAD),
                     [(partial(wq_copy, 1), 0, n_wq)])
    stream.start(WARMUP)
    stream.start(LEAD, queues=(1,))
    x_copy.start()
    wr_copy.start()
    stream.start()

    x_copy.wait()
    wr_copy.wait()
    x = x_s[0].astype(f32)
    xn = jnp.broadcast_to(_layernorm(x), (8, D)).astype(bf16)

    def head_round(j, _):
        stream = _Stream(kv_run(j, 0, LEAD, LEAD + 2 * n_kv), kv_run(j, 1, 0, 2 * n_kv))
        stream.start(n_kv)
        pl.when(j == 1)(lambda: q_proj(4, 8))
        pl.when(j >= 2)(lambda: values(j - 2))
        stream.start()

        @pl.when(j == 0)
        def _():
            landed(wq_s, sem_w.at[0])
            q_proj(0, 4)
        pl.when(j >= 1)(lambda: scores(j - 1))
    lax.fori_loop(0, H - 1, head_round, None)

    def rest(odd):
        return [(partial(wo_copy, odd), 0, n_wo), (partial(gu_copy, odd), 0, n_gu),
                (partial(wd_copy, odd), 0, n_wd)]

    stream = _Stream(kv_run(H - 1, 0, LEAD, 2 * n_kv) + rest(0) + [(tail_copy, 0, TAIL // TAIL_ROWS)],
                     kv_run(H - 1, 1, 0, 2 * n_kv) + rest(1))
    for work, h in ((values, H - 3), (scores, H - 2), (values, H - 2), (scores, H - 1), (values, H - 1)):
        stream.start(n_kv)
        work(h)
    stream.start(n_wo - 3 * n_kv + 32)

    landed(wo_s, sem_w.at[1])
    y = jnp.zeros((8, D), f32)
    for c in range(0, 2 * WO_SPLIT, 2):
        y = o_proj(c, c + 2, y)
        stream.start((n_gu + n_wd - 32) // 2 + 1)
    stream.start()

    hres = x + y[0:1, :]
    hn = _layernorm(hres)
    wr = wr_s[...].astype(f32).reshape(1, D)
    gate = jax.nn.sigmoid(jnp.sum(hn * wr, axis=-1, keepdims=True))
    hb = jnp.broadcast_to(hn, (8, D)).astype(bf16)

    landed(wg_s, sem_w.at[2])
    landed(wu_s, sem_w.at[3])
    g = jnp.dot(hb, wg_s[...].reshape(D, F), preferred_element_type=f32)
    u = jnp.dot(hb, wu_s[...].reshape(D, F), preferred_element_type=f32)
    gu = g * jax.nn.sigmoid(g) * u
    for r in range(0, TAIL, 128):
        c = gu[:1, 2 * half + r:2 * half + r + 128] * gate
        c_s[r:r + 128, :] = jnp.broadcast_to(c, (128, 128)).T
    gu = gu.astype(bf16)

    y = jnp.zeros((8, D), f32)
    for part, (r0, r1) in enumerate(((0, cut), (cut, half))):
        for odd in (0, 1):
            landed(wd_s.at[pl.ds(odd * half + r0, r1 - r0)], sem_d.at[2 * odd + part])
        for o in (0, half):
            y = y + jnp.dot(gu[:, o + r0:o + r1], wd_s[o + r0:o + r1, :],
                            preferred_element_type=f32)
    base = hres + (hn + y[:1] * gate)

    acc = jnp.zeros((8, D), f32)
    for j, r in enumerate(range(0, TAIL, TAIL_GROUP)):
        landed(wd_s.at[pl.ds(2 * half + r, TAIL_GROUP)], sem_t.at[j])
        w = wd_s[2 * half + r:2 * half + r + TAIL_GROUP, :].astype(f32)
        for t in range(0, TAIL_GROUP, 8):
            c = c_s[r + t:r + t + 8, :]
            acc = acc + w[t:t + 8, :] * jnp.concatenate([c] * (D // 128), axis=1)
    o_ref[0] = (base + jnp.sum(acc, axis=0, keepdims=True)).astype(o_ref.dtype)


@jax.jit
def pallas_sequential_preLN__sliding_block_cached__moe_arch_mod__decode_kernel(
    A_x: jax.Array,
    A_k_cache: jax.Array,
    A_v_cache: jax.Array,
    A_wq: jax.Array,
    A_wo: jax.Array,
    B_x: jax.Array,
    B_w_r: jax.Array,
    B_w_gate: jax.Array,
    B_w_up: jax.Array,
    B_w_down: jax.Array,
):
    del B_x
    _, H, Sk, Dh = A_k_cache.shape
    D = A_x.shape[-1]
    F = B_w_gate.shape[-1]
    W = min(4096, max(256, Sk // 4))
    kt = jnp.transpose(A_k_cache, (0, 1, 3, 2))
    vt = jnp.transpose(A_v_cache, (0, 1, 3, 2))
    wq = A_wq.reshape(WQ_SPLIT, D // WQ_SPLIT, H * Dh)
    wo = A_wo.reshape(WO_SPLIT, H * Dh // WO_SPLIT, D)
    wg = B_w_gate.reshape(GU_SPLIT, D // GU_SPLIT, F)
    wu = B_w_up.reshape(GU_SPLIT, D // GU_SPLIT, F)
    like = lambda a: pltpu.VMEM(a.shape, a.dtype)
    return pl.pallas_call(
        _kernel,
        out_shape=jax.ShapeDtypeStruct(A_x.shape, A_x.dtype),
        in_specs=[pl.BlockSpec(memory_space=pl.ANY)] * 9,
        scratch_shapes=[
            like(A_x), like(B_w_r), like(wq), like(wo), like(wg), like(wu), like(B_w_down),
            pltpu.VMEM((NBUF, Dh, W), A_k_cache.dtype),
            pltpu.VMEM((NBUF, Dh, W), A_v_cache.dtype),
            pltpu.VMEM((H, 8, Dh), jnp.bfloat16),
            pltpu.VMEM((8, W), jnp.bfloat16),
            pltpu.VMEM((8, 128), jnp.float32),
            pltpu.VMEM((8, Dh), jnp.float32),
            pltpu.VMEM((8, H * Dh), jnp.bfloat16),
            pltpu.VMEM((TAIL, 128), jnp.float32),
            pltpu.SemaphoreType.DMA((NBUF,)), pltpu.SemaphoreType.DMA((NBUF,)),
            pltpu.SemaphoreType.DMA((6,)), pltpu.SemaphoreType.DMA((4,)),
            pltpu.SemaphoreType.DMA((TAIL // TAIL_GROUP,)),
        ],
        compiler_params=pltpu.CompilerParams(
            vmem_limit_bytes=100 * 2**20,
            disable_bounds_checks=True, disable_semaphore_checks=True),
    )(A_x, kt, vt, wq, wo, B_w_r, wg, wu, B_w_down)
```

```python
from functools import partial

import jax
import jax.numpy as jnp
from jax import lax
import jax.experimental.pallas as pl
import jax.experimental.pallas.tpu as pltpu

EPS = 1e-5
LEAD = 26
WARMUP = 2
KV_ROWS, KV_COLS = 32, 512
NBUF = 4
WQ_SPLIT, WO_SPLIT, GU_SPLIT = 5, 3, 4
DOWN_ROWS = 32
TAIL = 256
TAIL_ROWS, TAIL_GROUP = 8, 16


def _layernorm(x):
    m = jnp.mean(x, axis=-1, keepdims=True)
    d = x - m
    v = jnp.mean(d * d, axis=-1, keepdims=True)
    return d / jnp.sqrt(v + EPS)


def _divmod(n, d, limit):
    if isinstance(n, int):
        return divmod(n, d)
    m = -(-(1 << 16) // d)
    assert all((i * m) >> 16 == i // d for i in range(limit))
    q = (n * m) >> 16
    return q, n - q * d


class _Stream:
    def __init__(self, low, high):
        self.todo = {1: list(low), 0: list(high)}

    def start(self, steps=1 << 30, queues=(1, 0), unroll=False):
        while steps > 0:
            live = [q for q in queues if self.todo[q]]
            if not live:
                return
            heads = {q: self.todo[q][0] for q in live}
            k = min([steps] + [end - first for _, first, end in heads.values()])

            def body(n, _, live=live, heads=heads):
                for q in live:
                    heads[q][0](heads[q][1] + n).start(priority=q)
            if unroll:
                for n in range(k):
                    body(n, None)
            else:
                lax.fori_loop(0, k, body, None)
            for q in live:
                copy, first, end = heads[q]
                if first + k < end:
                    self.todo[q][0] = (copy, first + k, end)
                else:
                    self.todo[q].pop(0)
            steps -= k


def _kernel(x_hbm, kt_hbm, vt_hbm, wq_hbm, wo_hbm, wr_hbm, wg_hbm, wu_hbm, wd_hbm,
            o_ref,
            x_s, wr_s, wq_s, wo_s, wg_s, wu_s, wd_s, k_s, v_s, q_s, p_s, l_s, even_s, o_s, c_s,
            sem_k, sem_v, sem_w, sem_d, sem_t):
    _, H, Dh, Sk = kt_hbm.shape
    W = k_s.shape[-1]
    D = x_hbm.shape[-1]
    F = wd_hbm.shape[0]
    f32, bf16 = jnp.float32, jnp.bfloat16

    def span(start, size):
        if isinstance(start, int):
            return pl.ds(start * size, size)
        return pl.ds(pl.multiple_of(start * size, size), size)

    per_col = Dh // KV_ROWS // 2
    n_kv = per_col * (W // KV_COLS)

    def kv_copy(which, h, odd, n):
        src, dst, sem = ((kt_hbm, k_s, sem_k), (vt_hbm, v_s, sem_v))[which]
        c, i = _divmod(n, per_col, n_kv)
        rows, slot = span(2 * i + odd, KV_ROWS), h & (NBUF - 1)
        return pltpu.make_async_copy(
            src.at[0, h, rows, span((Sk - W) // KV_COLS + c, KV_COLS)],
            dst.at[slot, rows, span(c, KV_COLS)], sem.at[slot])

    n_wq = 192

    def wq_copy(odd, n):
        a, b = _divmod(n, 3, n_wq)
        r, c = _divmod(b * 64 + a, 12, n_wq)
        idx = (pl.ds(4, 1) if odd else pl.ds(0, 4), span(r, 8), span(c, 512))
        return pltpu.make_async_copy(wq_hbm.at[idx], wq_s.at[idx], sem_w.at[0])

    n_wo = 256

    def wo_copy(odd, n):
        a, b = _divmod(n, 5, n_wo)
        r = jnp.where(a == 51, 153, b * 51 + a + jnp.where(b >= 3, 1, 0))
        idx = (pl.ds(2 * odd, 2 - odd), span(r, 8), slice(None))
        return pltpu.make_async_copy(wo_hbm.at[idx], wo_s.at[idx], sem_w.at[1])

    n_gu = 60

    def gu_copy(odd, n):
        src, dst = ((wg_hbm, wg_s), (wu_hbm, wu_s))[odd]
        r, c = _divmod(n, 3, n_gu)
        idx = (slice(None), span(r, 8), span(c, 512))
        return pltpu.make_async_copy(src.at[idx], dst.at[idx], sem_w.at[2 + odd])

    half = (F - TAIL) // 2
    cut = half - 128
    n_wd = half // DOWN_ROWS

    def wd_copy(odd, n):
        idx = (span(odd * n_wd + n, DOWN_ROWS), slice(None))
        part = jnp.where(n * DOWN_ROWS >= cut, 1, 0)
        return pltpu.make_async_copy(wd_hbm.at[idx], wd_s.at[idx], sem_d.at[2 * odd + part])

    def tail_copy(n):
        idx = (span(2 * half // TAIL_ROWS + n, TAIL_ROWS), slice(None))
        group = _divmod(n, TAIL_GROUP // TAIL_ROWS, TAIL // TAIL_ROWS)[0]
        return pltpu.make_async_copy(wd_hbm.at[idx], wd_s.at[idx], sem_t.at[group])

    def kv_run(h, odd, first, end):
        run = []
        while first < end:
            b, n = divmod(first, n_kv)
            k = min(n_kv - n, end - first)
            run.append((partial(kv_copy, b % 2, h + b // 2, odd), n, n + k))
            first += k
        return run

    def landed(dst, sem):
        pltpu.make_async_copy(dst, dst, sem).wait()

    def q_proj(g0, g1):
        def body(g, _):
            w = wq_s[:, :, span(g, 4 * Dh)].reshape(D, 4 * Dh)
            q = jnp.dot(xn, w, preferred_element_type=f32)
            for j in range(4):
                q_s[g * 4 + j] = q[:, j * Dh:(j + 1) * Dh].astype(bf16)
        lax.fori_loop(g0, g1, body, None)

    def scores(h):
        slot = h & (NBUF - 1)
        landed(k_s.at[slot], sem_k.at[slot])
        s = jnp.dot(q_s[h], k_s[slot], preferred_element_type=f32) * Dh ** -0.5
        e = jnp.exp(s - jnp.max(s, axis=-1, keepdims=True))
        l_s[...] = jnp.broadcast_to(jnp.sum(e, axis=-1, keepdims=True), l_s.shape)
        p_s[...] = e.astype(bf16)

    def values(h):
        slot = h & (NBUF - 1)
        landed(v_s.at[slot], sem_v.at[slot])
        a = lax.dot_general(p_s[...], v_s[slot], (((1,), (1,)), ((), ())),
                            preferred_element_type=f32)
        o = a / l_s[:, :1]

        @pl.when(h & 1 == 0)
        def _():
            even_s[...] = o

        @pl.when(h & 1 == 1)
        def _():
            o_s[:, span(h >> 1, 2 * Dh)] = jnp.concatenate([even_s[...], o], axis=1).astype(bf16)

    def o_proj(c0, c1, y):
        rows = wo_s.shape[1] // 2

        def body(c, y):
            return y + jnp.dot(o_s[:, span(c, rows)], wo_s[c >> 1, span(c & 1, rows), :],
                               preferred_element_type=f32)
        return lax.fori_loop(c0, c1, body, y)

    x_copy = pltpu.make_async_copy(x_hbm, x_s, sem_w.at[4])
    wr_copy = pltpu.make_async_copy(wr_hbm, wr_s, sem_w.at[5])

    stream = _Stream([(partial(wq_copy, 0), 0, n_wq)] + kv_run(0, 0, 0, LEAD),
                     [(partial(wq_copy, 1), 0, n_wq)])
    stream.start(WARMUP, unroll=True)
    stream.start(LEAD, queues=(1,), unroll=True)
    x_copy.start()
    wr_copy.start()
    stream.start()

    x_copy.wait()
    wr_copy.wait()
    x = x_s[0].astype(f32)
    xn = jnp.broadcast_to(_layernorm(x), (8, D)).astype(bf16)

    def head_round(j, _):
        stream = _Stream(kv_run(j, 0, LEAD, LEAD + 2 * n_kv), kv_run(j, 1, 0, 2 * n_kv))
        stream.start(n_kv)
        pl.when(j == 1)(lambda: q_proj(4, 8))
        pl.when(j >= 2)(lambda: values(j - 2))
        stream.start()

        @pl.when(j == 0)
        def _():
            landed(wq_s, sem_w.at[0])
            q_proj(0, 4)
        pl.when(j >= 1)(lambda: scores(j - 1))
    lax.fori_loop(0, H - 1, head_round, None)

    def rest(odd):
        return [(partial(wo_copy, odd), 0, n_wo), (partial(gu_copy, odd), 0, n_gu),
                (partial(wd_copy, odd), 0, n_wd)]

    stream = _Stream(kv_run(H - 1, 0, LEAD, 2 * n_kv) + rest(0) + [(tail_copy, 0, TAIL // TAIL_ROWS)],
                     kv_run(H - 1, 1, 0, 2 * n_kv) + rest(1))
    for work, h in ((values, H - 3), (scores, H - 2), (values, H - 2), (scores, H - 1), (values, H - 1)):
        stream.start(n_kv)
        work(h)
    stream.start(n_wo - 3 * n_kv + 32)

    landed(wo_s, sem_w.at[1])
    y = jnp.zeros((8, D), f32)
    for c in range(0, 2 * WO_SPLIT, 2):
        y = o_proj(c, c + 2, y)
        stream.start((n_gu + n_wd - 32) // 2 + 1)
    stream.start()

    hres = x + y[0:1, :]
    hn = _layernorm(hres)
    wr = wr_s[...].astype(f32).reshape(1, D)
    gate = jax.nn.sigmoid(jnp.sum(hn * wr, axis=-1, keepdims=True))
    hb = jnp.broadcast_to(hn, (8, D)).astype(bf16)

    landed(wg_s, sem_w.at[2])
    landed(wu_s, sem_w.at[3])
    g = jnp.dot(hb, wg_s[...].reshape(D, F), preferred_element_type=f32)
    u = jnp.dot(hb, wu_s[...].reshape(D, F), preferred_element_type=f32)
    gu = g * jax.nn.sigmoid(g) * u
    for r in range(0, TAIL, 128):
        c = gu[:1, 2 * half + r:2 * half + r + 128] * gate
        c_s[r:r + 128, :] = jnp.broadcast_to(c, (128, 128)).T
    gu = gu.astype(bf16)

    y = jnp.zeros((8, D), f32)
    for part, (r0, r1) in enumerate(((0, cut), (cut, half))):
        for odd in (0, 1):
            landed(wd_s.at[pl.ds(odd * half + r0, r1 - r0)], sem_d.at[2 * odd + part])
        for o in (0, half):
            y = y + jnp.dot(gu[:, o + r0:o + r1], wd_s[o + r0:o + r1, :],
                            preferred_element_type=f32)
    base = hres + (hn + y[:1] * gate)

    acc = jnp.zeros((8, D), f32)
    for j, r in enumerate(range(0, TAIL, TAIL_GROUP)):
        landed(wd_s.at[pl.ds(2 * half + r, TAIL_GROUP)], sem_t.at[j])
        w = wd_s[2 * half + r:2 * half + r + TAIL_GROUP, :].astype(f32)
        for t in range(0, TAIL_GROUP, 8):
            c = c_s[r + t:r + t + 8, :]
            acc = acc + w[t:t + 8, :] * jnp.concatenate([c] * (D // 128), axis=1)
    for j in range(D // 128):
        lanes = slice(j * 128, (j + 1) * 128)
        out = base[:, lanes] + jnp.sum(acc[:, lanes], axis=0, keepdims=True)
        o_ref[j] = out.astype(o_ref.dtype)


@jax.jit
def pallas_sequential_preLN__sliding_block_cached__moe_arch_mod__decode_kernel(
    A_x: jax.Array,
    A_k_cache: jax.Array,
    A_v_cache: jax.Array,
    A_wq: jax.Array,
    A_wo: jax.Array,
    B_x: jax.Array,
    B_w_r: jax.Array,
    B_w_gate: jax.Array,
    B_w_up: jax.Array,
    B_w_down: jax.Array,
):
    del B_x
    _, H, Sk, Dh = A_k_cache.shape
    D = A_x.shape[-1]
    F = B_w_gate.shape[-1]
    W = min(4096, max(256, Sk // 4))
    assert (H, Dh, D, F, W) == (32, 192, 640, 1536, 4096), "the copy schedule is laid out for these sizes"
    kt = jnp.transpose(A_k_cache, (0, 1, 3, 2))
    vt = jnp.transpose(A_v_cache, (0, 1, 3, 2))
    wq = A_wq.reshape(WQ_SPLIT, D // WQ_SPLIT, H * Dh)
    wo = A_wo.reshape(WO_SPLIT, H * Dh // WO_SPLIT, D)
    wg = B_w_gate.reshape(GU_SPLIT, D // GU_SPLIT, F)
    wu = B_w_up.reshape(GU_SPLIT, D // GU_SPLIT, F)
    like = lambda a: pltpu.VMEM(a.shape, a.dtype)
    out = pl.pallas_call(
        _kernel,
        out_shape=jax.ShapeDtypeStruct((D // 128, 1, 128), A_x.dtype),
        in_specs=[pl.BlockSpec(memory_space=pl.ANY)] * 9,
        scratch_shapes=[
            like(A_x), like(B_w_r), like(wq), like(wo), like(wg), like(wu), like(B_w_down),
            pltpu.VMEM((NBUF, Dh, W), A_k_cache.dtype),
            pltpu.VMEM((NBUF, Dh, W), A_v_cache.dtype),
            pltpu.VMEM((H, 8, Dh), jnp.bfloat16),
            pltpu.VMEM((8, W), jnp.bfloat16),
            pltpu.VMEM((8, 128), jnp.float32),
            pltpu.VMEM((8, Dh), jnp.float32),
            pltpu.VMEM((8, H * Dh), jnp.bfloat16),
            pltpu.VMEM((TAIL, 128), jnp.float32),
            pltpu.SemaphoreType.DMA((NBUF,)), pltpu.SemaphoreType.DMA((NBUF,)),
            pltpu.SemaphoreType.DMA((6,)), pltpu.SemaphoreType.DMA((4,)),
            pltpu.SemaphoreType.DMA((TAIL // TAIL_GROUP,)),
        ],
        compiler_params=pltpu.CompilerParams(
            vmem_limit_bytes=100 * 2**20,
            disable_bounds_checks=True, disable_semaphore_checks=True),
    )(A_x, kt, vt, wq, wo, B_w_r, wg, wu, B_w_down)
    return out.reshape(A_x.shape)
```
